```python
import jax
import jax.numpy as jnp

def _softmax(x, axis=-1):
    return jax.nn.softmax(x, axis=axis)

def _gelu(x):
    return jax.nn.gelu(x, approximate=True)

def _silu(x):
    return jax.nn.silu(x)

def _sigmoid(x):
    return jax.nn.sigmoid(x)

def _layernorm(x, axis=-1, eps=1e-05):
    m = jnp.mean(x, axis=axis, keepdims=True)
    v = jnp.var(x, axis=axis, keepdims=True)
    return (x - m) / jnp.sqrt(v + eps)

def _scatter_add(tgt, idx, src, axis=0):
    return tgt.at[idx].add(src)

def _segment_sum(src, seg, n):
    return jax.ops.segment_sum(src, seg, n)

class _Rng:

    def __init__(self, key):
        self._k = key

    def _next(self):
        self._k, sub = jax.random.split(self._k)
        return sub

    def normal(self, shape):
        return jax.random.normal(self._next(), shape, dtype=jnp.bfloat16)

    def randint(self, lo, hi, shape):
        return jax.random.randint(self._next(), shape, lo, hi, dtype=jnp.int32)

    def uniform(self, shape, lo=0.0, hi=1.0):
        return jax.random.uniform(self._next(), shape, jnp.bfloat16, lo, hi)

    def permutation(self, n):
        return jax.random.permutation(self._next(), n)
kernel_name = 'standalone__dilated_atrous__vision'

def setup_inputs():
    _rng = _Rng(jax.random.key(int.from_bytes(__import__("os").urandom(4), "little")))
    _w = lambda a: (lambda t: t.astype(jnp.bfloat16) if jnp.issubdtype(t.dtype, jnp.floating) else t)(jnp.asarray(a))
    H = W = 384
    C = 384
    k = 1
    return {'x': _w((lambda *s: _rng.normal(s) * 0.05)(1, H, W, C)), 'w': _w((lambda *s: _rng.normal(s) * 0.05)(k, k, C, C) * (1.0 / (k * C ** 0.5)))}

def reference(x, w):
    B, H, W, C = x.shape
    k = 1
    rate = 2
    pad = (k - 1) * rate // 2
    xp = jnp.pad(x, ((0, 0), (pad, pad), (pad, pad), (0, 0)))
    out = jnp.zeros_like(x)
    for i in range(k):
        for j in range(k):
            tap = xp[:, i * rate:i * rate + H, j * rate:j * rate + W, :].copy()
            out = out + jnp.einsum('bhwc,co->bhwo', tap, w[i, j])
    return out
```

```python
import jax
import jax.numpy as jnp
from jax import lax
import jax.experimental.pallas as pl
import jax.experimental.pallas.tpu as pltpu

_GROUPS, _SLABS = 6, 6
_PIECE = 128
_STEP = 768
_LAG = 5
_LATE = 3
_W_ROWS = 96
_W_FIRST = 30
_W_PER_STEP = 14


def _upper(shape):
    return lax.broadcasted_iota(jnp.int32, shape, 1) < 4


def _tiles_to_rows(v):
    n = v.shape[0] // 48
    u = pltpu.bitcast(v, jnp.int32).reshape(n, 24, 128)
    a, b, c = u[:, 0:8], u[:, 8:16], u[:, 16:24]
    up = _upper(a.shape)
    cols = [jnp.where(up, a, b), pltpu.roll(jnp.where(up, c, a), 4, 1), jnp.where(up, b, c)]
    return jnp.concatenate(
        [pltpu.bitcast(t.reshape(8 * n, 128), v.dtype) for t in cols], axis=1)


def _rows_to_tiles(r):
    n = r.shape[0] // 16
    c0, c1, c2 = (
        pltpu.bitcast(r[:, i * 128:(i + 1) * 128], jnp.int32).reshape(n, 8, 128)
        for i in range(3))
    up = _upper(c0.shape)
    c1 = pltpu.roll(c1, 4, 1)
    u = jnp.concatenate(
        [jnp.where(up, c0, c1), jnp.where(up, c2, c0), jnp.where(up, c1, c2)], axis=1)
    return pltpu.bitcast(u.reshape(24 * n, 128), r.dtype)


@jax.jit
def pallas_standalone__dilated_atrous__vision_kernel(
    x: jax.Array,
    w: jax.Array,
):
    B, H, W, C = x.shape
    assert w.shape == (1, 1, C, C) and C == 3 * 128 and x.dtype.itemsize == 2
    M = B * H * W
    n_slabs = _GROUPS * _SLABS
    slab_rows = 3 * M // n_slabs
    half = slab_rows // 2
    group_rounds = half // _PIECE
    group_steps = slab_rows // _STEP
    group_writes = slab_rows // _W_ROWS
    n_batches = _GROUPS * group_rounds // _SLABS
    n_steps = _GROUPS * group_steps
    n_writes = _GROUPS * group_writes
    step_writes = group_writes // group_steps
    assert n_slabs * slab_rows == 3 * M and group_rounds * _PIECE * 2 == slab_rows
    assert group_steps * _STEP == slab_rows and step_writes * group_steps == group_writes
    assert _STEP == _SLABS * _PIECE and 2 * n_batches == n_steps
    assert _LAG <= _SLABS and _LAG * _SLABS <= _W_FIRST <= (n_batches - _LATE) * step_writes

    def kernel_function(x_hbm, w_hbm, o_hbm, buf, wbuf, out_sem):
        def write(k):
            g = lax.div(k, group_writes)
            slabs = pl.ds(g * _SLABS, _SLABS)
            rows = pl.ds(pl.multiple_of((k - g * group_writes) * _W_ROWS, _W_ROWS), _W_ROWS)
            return pltpu.make_async_copy(
                buf.at[slabs, rows], o_hbm.at[slabs, rows], out_sem)

        def start_writes(lo, hi):
            lax.fori_loop(lo, hi, lambda k, _: write(k).start(priority=1), None)

        def matmul_step(i, between=lambda s: None):
            g = lax.div(i, group_steps)
            rows = pl.ds(pl.multiple_of((i - g * group_steps) * _STEP, _STEP), _STEP)
            nxt = _tiles_to_rows(buf[g * _SLABS, rows])
            for s in range(_SLABS):
                res = jnp.dot(nxt, wbuf[...], preferred_element_type=jnp.float32)
                if s + 1 < _SLABS:
                    nxt = _tiles_to_rows(buf[g * _SLABS + s + 1, rows])
                between(s)
                buf[g * _SLABS + s, rows] = _rows_to_tiles(res.astype(buf.dtype))

        def phases(sems, w_sem):
            def batch_sem(b):
                return sems.at[lax.rem(b, _LATE + 1)]

            def read(rnd, second_half, s):
                g = lax.div(rnd, group_rounds)
                row = second_half * half + (rnd - g * group_rounds) * _PIECE
                idx = (g * _SLABS + s, pl.ds(pl.multiple_of(row, _PIECE), _PIECE))
                return pltpu.make_async_copy(
                    x_hbm.at[idx], buf.at[idx], batch_sem(lax.div(rnd, _SLABS)))

            def start_round(rnd, both=True):
                for s in range(_SLABS):
                    read(rnd, 0, s).start(priority=1)
                    if both:
                        read(rnd - _LAG, 1, s).start(priority=0)

            def wait_batch(b):
                total = buf.at[pl.ds(0, _SLABS), pl.ds(0, 2 * _STEP)]
                pltpu.make_async_copy(total, total, batch_sem(b)).wait()

            w_copy = pltpu.make_async_copy(w_hbm, wbuf, w_sem)
            w_copy.start()
            lax.fori_loop(0, _LAG, lambda r, _: start_round(r, both=False), None)
            lax.fori_loop(_LAG, _LATE * _SLABS, lambda r, _: start_round(r), None)
            w_copy.wait()

            def read_step(i, _):
                wait_batch(i - _LATE)
                matmul_step(i - _LATE, lambda s: start_round(i * _SLABS + s))

            lax.fori_loop(_LATE, n_batches, read_step, None)

            def hand_off(r, _):
                for s in range(_SLABS):
                    write(r * _SLABS + s).start(priority=1)
                    read(n_batches * _SLABS + r - _LAG, 1, s).start(priority=0)

            lax.fori_loop(0, _LAG, hand_off, None)
            start_writes(_LAG * _SLABS, _W_FIRST)

            def write_step(i, started):
                @pl.when(i < n_batches + _LATE)
                def _():
                    wait_batch(i - _LATE)

                ready = (i - _LATE) * step_writes
                target = jnp.minimum(ready, _W_FIRST + (i - n_batches) * _W_PER_STEP)
                start_writes(started, target)
                matmul_step(i - _LATE)
                return target

            started = lax.fori_loop(
                n_batches, n_steps + _LATE, write_step, jnp.int32(_W_FIRST))
            start_writes(started, n_writes)

        pl.run_scoped(
            phases,
            pltpu.SemaphoreType.DMA((_LATE + 1,)),
            pltpu.SemaphoreType.DMA(()),
        )
        pltpu.make_async_copy(buf, o_hbm, out_sem).wait()

    tiles = x.reshape(M // 8, 8, 3, 128).transpose(0, 2, 1, 3)
    out = pl.pallas_call(
        kernel_function,
        in_specs=[
            pl.BlockSpec(memory_space=pl.ANY),
            pl.BlockSpec(memory_space=pl.ANY),
        ],
        out_specs=pl.BlockSpec(memory_space=pl.ANY),
        out_shape=jax.ShapeDtypeStruct((n_slabs, slab_rows, 128), x.dtype),
        scratch_shapes=[
            pltpu.VMEM((n_slabs, slab_rows, 128), x.dtype),
            pltpu.VMEM((C, C), w.dtype),
            pltpu.SemaphoreType.DMA(()),
        ],
        compiler_params=pltpu.CompilerParams(
            vmem_limit_bytes=120 * 2**20, disable_bounds_checks=True),
    )(tiles.reshape(n_slabs, slab_rows, 128), w.reshape(C, C))
    return out.reshape(M // 8, 3, 8, 128).transpose(0, 2, 1, 3).reshape(B, H, W, C)
```

```python
import jax
import jax.numpy as jnp
from jax import lax
import jax.experimental.pallas as pl
import jax.experimental.pallas.tpu as pltpu

_R_STREAMS = 12
_R_STRIDE = 6144
_R_PIECE = 128
_CHUNKS = 6
_CHUNK = 768
_LATE = 3
_W_STREAMS = 6
_W_STRIDE = 4096
_W_PIECE = 64
_W_FIRST = 40
_W_PER_STEP = 20


def _upper(shape):
    return lax.broadcasted_iota(jnp.int32, shape, 1) < 4


def _tiles_to_rows(v):
    n = v.shape[0] // 48
    u = pltpu.bitcast(v, jnp.int32).reshape(n, 24, 128)
    a, b, c = u[:, 0:8], u[:, 8:16], u[:, 16:24]
    up = _upper(a.shape)
    cols = [jnp.where(up, a, b), pltpu.roll(jnp.where(up, c, a), 4, 1), jnp.where(up, b, c)]
    return jnp.concatenate(
        [pltpu.bitcast(t.reshape(8 * n, 128), v.dtype) for t in cols], axis=1)


def _rows_to_tiles(r):
    n = r.shape[0] // 16
    c0, c1, c2 = (
        pltpu.bitcast(r[:, i * 128:(i + 1) * 128], jnp.int32).reshape(n, 8, 128)
        for i in range(3))
    up = _upper(c0.shape)
    c1 = pltpu.roll(c1, 4, 1)
    u = jnp.concatenate(
        [jnp.where(up, c0, c1), jnp.where(up, c2, c0), jnp.where(up, c1, c2)], axis=1)
    return pltpu.bitcast(u.reshape(24 * n, 128), r.dtype)


@jax.jit
def pallas_standalone__dilated_atrous__vision_kernel(
    x: jax.Array,
    w: jax.Array,
):
    B, H, W, C = x.shape
    assert w.shape == (1, 1, C, C) and C == 3 * 128 and x.dtype.itemsize == 2
    M = B * H * W
    N = 3 * M
    block = _R_STREAMS * _R_STRIDE
    block_rounds = _R_STRIDE // _R_PIECE
    step_rows = _CHUNKS * _CHUNK
    block_steps = block // step_rows
    n_batches = N // block * block_rounds // _CHUNKS
    n_steps = N // step_rows
    group = _W_STREAMS * _W_STRIDE
    group_writes = _W_STRIDE // _W_PIECE
    n_writes = N // group * group_writes
    assert N % block == 0 and N % group == 0 and _CHUNK % 48 == 0
    assert block_steps * step_rows == block and block_rounds % _CHUNKS == 0
    assert _CHUNK == _CHUNKS * _R_PIECE and _R_STREAMS % _CHUNKS == 0
    assert block_steps >= 2 * block_rounds // _CHUNKS - 1
    assert n_batches - _LATE >= block_steps and block >= group and _W_FIRST <= group_writes

    def kernel_function(x_hbm, w_hbm, o_hbm, buf, wbuf, out_sem):
        slabs = buf.reshape(N // _W_STRIDE, _W_STRIDE, 128)

        def write(k):
            g = lax.div(k, group_writes)
            row = pl.multiple_of((k - g * group_writes) * _W_PIECE, _W_PIECE)
            idx = (pl.ds(g * _W_STREAMS, _W_STREAMS), pl.ds(row, _W_PIECE))
            return pltpu.make_async_copy(slabs.at[idx], o_hbm.at[idx], out_sem)

        def start_writes(lo, hi):
            lax.fori_loop(lo, hi, lambda k, _: write(k).start(priority=1), None)

        def matmul_step(i, between=lambda s: None):
            first = i < block_steps
            base = jnp.where(first, i * _CHUNK, i * step_rows)
            stride = jnp.where(first, block // _CHUNKS, _CHUNK)

            def rows(s):
                return pl.ds(pl.multiple_of(base + s * stride, _CHUNK), _CHUNK)

            nxt = _tiles_to_rows(buf[rows(0)])
            for s in range(_CHUNKS):
                res = jnp.dot(nxt, wbuf[...], preferred_element_type=jnp.float32)
                if s + 1 < _CHUNKS:
                    nxt = _tiles_to_rows(buf[rows(s + 1)])
                between(s)
                buf[rows(s)] = _rows_to_tiles(res.astype(buf.dtype))

        def phases(sems, w_sem):
            def batch_sem(b):
                return sems.at[lax.rem(b, _LATE + 1)]

            def start_round(r):
                g = lax.div(r, block_rounds)
                row = g * block + (r - g * block_rounds) * _R_PIECE
                sem = batch_sem(lax.div(r, _CHUNKS))
                for s in range(_R_STREAMS):
                    rows = pl.ds(pl.multiple_of(row + s * _R_STRIDE, _R_PIECE), _R_PIECE)
                    copy = pltpu.make_async_copy(x_hbm.at[rows], buf.at[rows], sem)
                    copy.start(priority=1 - s % 2)

            def wait_batch(b):
                total = buf.at[pl.ds(0, _CHUNKS * _R_STREAMS * _R_PIECE)]
                pltpu.make_async_copy(total, total, batch_sem(b)).wait()

            w_copy = pltpu.make_async_copy(w_hbm, wbuf, w_sem)
            w_copy.start()
            lax.fori_loop(0, _LATE * _CHUNKS, lambda r, _: start_round(r), None)
            w_copy.wait()

            def read_step(i, _):
                wait_batch(i - _LATE)
                matmul_step(i - _LATE, lambda s: start_round(i * _CHUNKS + s))

            lax.fori_loop(_LATE, n_batches, read_step, None)

            start_writes(0, _W_FIRST)

            def write_step(i, started):
                @pl.when(i < n_batches + _LATE)
                def _():
                    wait_batch(i - _LATE)

                ready = lax.div((i - _LATE) * step_rows, group) * group_writes
                target = jnp.minimum(ready, _W_FIRST + (i - n_batches) * _W_PER_STEP)
                start_writes(started, target)
                matmul_step(i - _LATE)
                return target

            started = lax.fori_loop(
                n_batches, n_steps + _LATE, write_step, jnp.int32(_W_FIRST))
            start_writes(started, n_writes)

        pl.run_scoped(
            phases,
            pltpu.SemaphoreType.DMA((_LATE + 1,)),
            pltpu.SemaphoreType.DMA(()),
        )
        pltpu.make_async_copy(slabs, o_hbm, out_sem).wait()

    tiles = x.reshape(M // 8, 8, 3, 128).transpose(0, 2, 1, 3).reshape(N, 128)
    out = pl.pallas_call(
        kernel_function,
        in_specs=[
            pl.BlockSpec(memory_space=pl.ANY),
            pl.BlockSpec(memory_space=pl.ANY),
        ],
        out_specs=pl.BlockSpec(memory_space=pl.ANY),
        out_shape=jax.ShapeDtypeStruct((N // _W_STRIDE, _W_STRIDE, 128), x.dtype),
        scratch_shapes=[
            pltpu.VMEM((N, 128), x.dtype),
            pltpu.VMEM((C, C), w.dtype),
            pltpu.SemaphoreType.DMA(()),
        ],
        compiler_params=pltpu.CompilerParams(
            vmem_limit_bytes=120 * 2**20, disable_bounds_checks=True),
    )(tiles, w.reshape(C, C))
    return out.reshape(M // 8, 3, 8, 128).transpose(0, 2, 1, 3).reshape(B, H, W, C)
```

```python
import jax
import jax.numpy as jnp
from jax import lax
import jax.experimental.pallas as pl
import jax.experimental.pallas.tpu as pltpu

_SLAB = 2048
_R_STREAMS = 12
_R_PIECE = 64
_R_LAG = 4
_R_TAIL = 10
_W_STREAMS = 6
_W_PIECE = 32
_W_FIRST = 40
_CHUNK = 384
_R_HEAD = 42
_R_STEP = (7, 6)
_W_STEP = (8, 26)


def _upper(shape):
    return lax.broadcasted_iota(jnp.int32, shape, 1) < 4


def _words_to_pixels(u, dtype):
    n = u.shape[0] // 24
    u = u.reshape(n, 24, 128)
    a, b, c = u[:, 0:8], u[:, 8:16], u[:, 16:24]
    up = _upper(a.shape)
    cols = [jnp.where(up, a, b), pltpu.roll(jnp.where(up, c, a), 4, 1), jnp.where(up, b, c)]
    return jnp.concatenate(
        [pltpu.bitcast(t.reshape(8 * n, 128), dtype) for t in cols], axis=1)


def _pixels_to_words(r):
    n = r.shape[0] // 16
    c0, c1, c2 = (
        pltpu.bitcast(r[:, i * 128:(i + 1) * 128], jnp.int32).reshape(n, 8, 128)
        for i in range(3))
    up = _upper(c0.shape)
    c1 = pltpu.roll(c1, 4, 1)
    u = jnp.concatenate(
        [jnp.where(up, c0, c1), jnp.where(up, c2, c0), jnp.where(up, c1, c2)], axis=1)
    return u.reshape(24 * n, 128)


def _share(total, parts, i):
    return range(i * total // parts, (i + 1) * total // parts)


@jax.jit
def pallas_standalone__dilated_atrous__vision_kernel(
    x: jax.Array,
    w: jax.Array,
):
    B, H, W, C = x.shape
    assert w.shape == (1, 1, C, C) and C == 3 * 128 and x.dtype.itemsize == 2
    M = B * H * W
    N = 3 * M // 2
    block = _R_STREAMS * _SLAB
    block_rounds = _SLAB // _R_PIECE
    n_blocks = N // block
    n_rounds = n_blocks * block_rounds
    group = _W_STREAMS * _SLAB
    group_writes = _SLAB // _W_PIECE
    n_writes = N // group * group_writes
    r_chunks, r_rounds = _R_STEP
    w_chunks, w_writes = _W_STEP
    r_steps = (n_rounds - _R_HEAD) // r_rounds - 1
    r_rows = r_steps * r_chunks * _CHUNK
    w_steps = (N - r_rows) // (w_chunks * _CHUNK)
    assert n_blocks * block == N and N % group == 0 and _CHUNK % 24 == 0
    assert r_rows + w_steps * w_chunks * _CHUNK == N and r_chunks * _CHUNK <= block
    assert _R_TAIL <= min(r_rounds, block_rounds) * _R_STREAMS // 2
    for t in range(w_steps):
        done = r_rows + t * w_chunks * _CHUNK
        assert _W_FIRST + (t + 1) * w_writes <= done // group * group_writes

    def kernel_function(x_hbm, w_hbm, o_hbm, buf, wbuf, wwords):
        x_hbm, o_hbm = x_hbm.bitcast(jnp.int32), o_hbm.bitcast(jnp.int32)
        slabs = buf.reshape(N // _SLAB, _SLAB, 128)

        def matmuls(base, count, between):
            def rows(s):
                return pl.ds(pl.multiple_of(base + s * _CHUNK, _CHUNK), _CHUNK)

            nxt = _words_to_pixels(buf[rows(0)], x.dtype)
            for s in range(count):
                wv = pltpu.bitcast(wwords[...], w.dtype)
                res = jnp.dot(nxt, wv, preferred_element_type=jnp.float32)
                if s + 1 < count:
                    nxt = _words_to_pixels(buf[rows(s + 1)], x.dtype)
                between(s)
                buf[rows(s)] = _pixels_to_words(res.astype(x.dtype))

        def wait_rows(rows, sem):
            total = buf.at[pl.ds(0, rows)]
            pltpu.make_async_copy(total, total, sem).wait()

        def phases(block_sems, side_sem, out_sem):
            def start_read(r, s, sem=None):
                queue = 1 - s % 2
                r = r if queue else r - _R_LAG
                g = lax.div(r, block_rounds)
                row = g * block + (r - g * block_rounds) * _R_PIECE + s * _SLAB
                rows = pl.ds(pl.multiple_of(row, _R_PIECE), _R_PIECE)
                sem = block_sems.at[g] if sem is None else sem
                copy = pltpu.make_async_copy(x_hbm.at[rows], buf.at[rows], sem)
                copy.start(priority=queue)

            def start_rounds(lo, hi, streams):
                @pl.loop(lo, hi)
                def _(r):
                    for s in streams:
                        start_read(r, s)

            def start_write(k):
                g = lax.div(k, group_writes)
                row = pl.multiple_of((k - g * group_writes) * _W_PIECE, _W_PIECE)
                idx = (pl.ds(g * _W_STREAMS, _W_STREAMS), pl.ds(row, _W_PIECE))
                pltpu.make_async_copy(slabs.at[idx], o_hbm.at[idx], out_sem).start(priority=1)

            w_copy = pltpu.make_async_copy(w_hbm, wbuf, side_sem)
            w_copy.start()
            start_rounds(0, _R_LAG, range(0, _R_STREAMS, 2))
            start_rounds(_R_LAG, _R_HEAD, range(_R_STREAMS))
            w_copy.wait()
            wwords[...] = pltpu.bitcast(wbuf[...], jnp.int32)
            wait_rows(block, block_sems.at[0])

            @pl.loop(0, r_steps)
            def _(i):
                base = i * (r_chunks * _CHUNK)
                g = lax.div(base + r_chunks * _CHUNK - 1, block)

                @pl.when(g * block >= jnp.maximum(base, 1))
                def _():
                    wait_rows(block, block_sems.at[g])

                def between(s):
                    for k in _share(r_rounds * _R_STREAMS, r_chunks, s):
                        r, stream = divmod(k, _R_STREAMS)
                        start_read(_R_HEAD + i * r_rounds + r, stream)

                matmuls(base, r_chunks, between)

            for r in range(_R_HEAD + r_steps * r_rounds, n_rounds):
                for s in range(_R_STREAMS):
                    left = ((n_rounds - r) * _R_STREAMS - s) // 2
                    in_tail = s % 2 == 0 and left <= _R_TAIL
                    start_read(jnp.int32(r), s, side_sem if in_tail else None)
            start_rounds(n_rounds, n_rounds + _R_LAG, range(1, _R_STREAMS, 2))
            for g in range((r_rows - 1) // block + 1, n_blocks - 1):
                wait_rows(block, block_sems.at[g])
            wait_rows(block - _R_TAIL * _R_PIECE, block_sems.at[n_blocks - 1])
            pl.loop(0, _W_FIRST)(start_write)
            wait_rows(_R_TAIL * _R_PIECE, side_sem)

            @pl.loop(0, w_steps)
            def _(t):
                def between(s):
                    for k in _share(w_writes, w_chunks, s):
                        start_write(_W_FIRST + t * w_writes + k)

                matmuls(r_rows + t * (w_chunks * _CHUNK), w_chunks, between)

            pl.loop(_W_FIRST + w_steps * w_writes, n_writes)(start_write)
            pltpu.make_async_copy(slabs, o_hbm, out_sem).wait()

        pl.run_scoped(
            phases,
            pltpu.SemaphoreType.DMA((n_blocks,)),
            pltpu.SemaphoreType.DMA(()),
            pltpu.SemaphoreType.DMA(()),
        )

    tiles = x.reshape(M // 8, 8, 3, 128).transpose(0, 2, 1, 3).reshape(2 * N, 128)
    out = pl.pallas_call(
        kernel_function,
        in_specs=[
            pl.BlockSpec(memory_space=pl.ANY),
            pl.BlockSpec(memory_space=pl.ANY),
        ],
        out_specs=pl.BlockSpec(memory_space=pl.ANY),
        out_shape=jax.ShapeDtypeStruct((N // _SLAB, 2 * _SLAB, 128), x.dtype),
        scratch_shapes=[
            pltpu.VMEM((N, 128), jnp.int32),
            pltpu.VMEM((C, C), w.dtype),
            pltpu.VMEM((C // 2, C), jnp.int32),
        ],
        compiler_params=pltpu.CompilerParams(
            vmem_limit_bytes=120 * 2**20, disable_bounds_checks=True),
    )(tiles, w.reshape(C, C))
    return out.reshape(M // 8, 3, 8, 128).transpose(0, 2, 1, 3).reshape(B, H, W, C)
```

```python
import jax
import jax.numpy as jnp
from jax import lax
import jax.experimental.pallas as pl
import jax.experimental.pallas.tpu as pltpu

_SLAB = 4096
_R_STREAMS = 12
_R_PIECE = 128
_R_LAG = 4
_R_TAIL = 10
_W_STREAMS = 6
_W_PIECE = 64
_W_FIRST = 40
_CHUNK = 768
_R_HEAD = 42
_R_STEP = (13, 12)
_W_STEP = (4, 13)


def _upper(shape):
    return lax.broadcasted_iota(jnp.int32, shape, 1) < 4


def _tiles_to_pixels(v):
    n = v.shape[0] // 48
    u = pltpu.bitcast(v, jnp.int32).reshape(n, 24, 128)
    a, b, c = u[:, 0:8], u[:, 8:16], u[:, 16:24]
    up = _upper(a.shape)
    cols = [jnp.where(up, a, b), pltpu.roll(jnp.where(up, c, a), 4, 1), jnp.where(up, b, c)]
    return jnp.concatenate(
        [pltpu.bitcast(t.reshape(8 * n, 128), v.dtype) for t in cols], axis=1)


def _pixels_to_tiles(r):
    n = r.shape[0] // 16
    c0, c1, c2 = (
        pltpu.bitcast(r[:, i * 128:(i + 1) * 128], jnp.int32).reshape(n, 8, 128)
        for i in range(3))
    up = _upper(c0.shape)
    c1 = pltpu.roll(c1, 4, 1)
    u = jnp.concatenate(
        [jnp.where(up, c0, c1), jnp.where(up, c2, c0), jnp.where(up, c1, c2)], axis=1)
    return pltpu.bitcast(u.reshape(24 * n, 128), r.dtype)


def _share(total, parts, i):
    return range(i * total // parts, (i + 1) * total // parts)


@jax.jit
def pallas_standalone__dilated_atrous__vision_kernel(
    x: jax.Array,
    w: jax.Array,
):
    B, H, W, C = x.shape
    assert w.shape == (1, 1, C, C) and C == 3 * 128 and x.dtype.itemsize == 2
    M = B * H * W
    N = 3 * M
    block = _R_STREAMS * _SLAB
    block_rounds = _SLAB // _R_PIECE
    n_blocks = N // block
    n_rounds = n_blocks * block_rounds
    group = _W_STREAMS * _SLAB
    group_writes = _SLAB // _W_PIECE
    n_writes = N // group * group_writes
    r_chunks, r_rounds = _R_STEP
    w_chunks, w_writes = _W_STEP
    r_steps = (n_rounds - _R_HEAD - 1) // r_rounds
    r_rows = r_steps * r_chunks * _CHUNK
    w_steps = (N - r_rows) // (w_chunks * _CHUNK)
    assert n_blocks * block == N and N % group == 0 and _CHUNK % 48 == 0
    assert r_rows + w_steps * w_chunks * _CHUNK == N and r_chunks * _CHUNK <= block
    assert 2 * _R_TAIL <= (n_rounds - _R_HEAD - r_steps * r_rounds) * _R_STREAMS
    for t in range(w_steps):
        done = r_rows + t * w_chunks * _CHUNK
        assert _W_FIRST + (t + 1) * w_writes <= done // group * group_writes

    def kernel_function(x_hbm, w_hbm, o_hbm, buf, wbuf):
        slabs = buf.reshape(N // _SLAB, _SLAB, 128)

        def matmuls(base, count, between):
            def rows(s):
                return pl.ds(pl.multiple_of(base + s * _CHUNK, _CHUNK), _CHUNK)

            nxt = _tiles_to_pixels(buf[rows(0)])
            for s in range(count):
                res = jnp.dot(nxt, wbuf[...], preferred_element_type=jnp.float32)
                if s + 1 < count:
                    nxt = _tiles_to_pixels(buf[rows(s + 1)])
                between(s)
                buf[rows(s)] = _pixels_to_tiles(res.astype(buf.dtype))

        def wait_rows(rows, sem):
            total = buf.at[pl.ds(0, rows)]
            pltpu.make_async_copy(total, total, sem).wait()

        def phases(block_sems, side_sem, out_sem):
            def start_read(r, s, sem=None):
                queue = 1 - s % 2
                r = r if queue else r - _R_LAG
                g = lax.div(r, block_rounds)
                row = g * block + (r - g * block_rounds) * _R_PIECE + s * _SLAB
                rows = pl.ds(pl.multiple_of(row, _R_PIECE), _R_PIECE)
                sem = block_sems.at[g] if sem is None else sem
                copy = pltpu.make_async_copy(x_hbm.at[rows], buf.at[rows], sem)
                copy.start(priority=queue)

            def start_rounds(lo, hi, streams):
                @pl.loop(lo, hi)
                def _(r):
                    for s in streams:
                        start_read(r, s)

            def start_write(k):
                g = lax.div(k, group_writes)
                row = pl.multiple_of((k - g * group_writes) * _W_PIECE, _W_PIECE)
                idx = (pl.ds(g * _W_STREAMS, _W_STREAMS), pl.ds(row, _W_PIECE))
                pltpu.make_async_copy(slabs.at[idx], o_hbm.at[idx], out_sem).start(priority=1)

            w_copy = pltpu.make_async_copy(w_hbm, wbuf, side_sem)
            w_copy.start()
            start_rounds(0, _R_LAG, range(0, _R_STREAMS, 2))
            start_rounds(_R_LAG, _R_HEAD, range(_R_STREAMS))
            w_copy.wait()
            wait_rows(block, block_sems.at[0])

            @pl.loop(0, r_steps)
            def _(i):
                base = i * (r_chunks * _CHUNK)
                g = lax.div(base + r_chunks * _CHUNK - 1, block)

                @pl.when(g * block >= jnp.maximum(base, 1))
                def _():
                    wait_rows(block, block_sems.at[g])

                def between(s):
                    for k in _share(r_rounds * _R_STREAMS, r_chunks, s):
                        r, stream = divmod(k, _R_STREAMS)
                        start_read(_R_HEAD + i * r_rounds + r, stream)

                matmuls(base, r_chunks, between)

            for r in range(_R_HEAD + r_steps * r_rounds, n_rounds):
                for s in range(_R_STREAMS):
                    left = ((n_rounds - r) * _R_STREAMS - s) // 2
                    in_tail = s % 2 == 0 and left <= _R_TAIL
                    start_read(jnp.int32(r), s, side_sem if in_tail else None)
            start_rounds(n_rounds, n_rounds + _R_LAG, range(1, _R_STREAMS, 2))
            for g in range((r_rows - 1) // block + 1, n_blocks - 1):
                wait_rows(block, block_sems.at[g])
            wait_rows(block - _R_TAIL * _R_PIECE, block_sems.at[n_blocks - 1])
            pl.loop(0, _W_FIRST)(start_write)
            wait_rows(_R_TAIL * _R_PIECE, side_sem)

            @pl.loop(0, w_steps)
            def _(t):
                def between(s):
                    for k in _share(w_writes, w_chunks, s):
                        start_write(_W_FIRST + t * w_writes + k)

                matmuls(r_rows + t * (w_chunks * _CHUNK), w_chunks, between)

            pl.loop(_W_FIRST + w_steps * w_writes, n_writes)(start_write)
            pltpu.make_async_copy(slabs, o_hbm, out_sem).wait()

        pl.run_scoped(
            phases,
            pltpu.SemaphoreType.DMA((n_blocks,)),
            pltpu.SemaphoreType.DMA(()),
            pltpu.SemaphoreType.DMA(()),
        )

    tiles = x.reshape(M // 8, 8, 3, 128).transpose(0, 2, 1, 3).reshape(N, 128)
    out = pl.pallas_call(
        kernel_function,
        in_specs=[
            pl.BlockSpec(memory_space=pl.ANY),
            pl.BlockSpec(memory_space=pl.ANY),
        ],
        out_specs=pl.BlockSpec(memory_space=pl.ANY),
        out_shape=jax.ShapeDtypeStruct((N // _SLAB, _SLAB, 128), x.dtype),
        scratch_shapes=[
            pltpu.VMEM((N, 128), x.dtype),
            pltpu.VMEM((C, C), w.dtype),
        ],
        compiler_params=pltpu.CompilerParams(
            vmem_limit_bytes=120 * 2**20, disable_bounds_checks=True),
    )(tiles, w.reshape(C, C))
    return out.reshape(M // 8, 3, 8, 128).transpose(0, 2, 1, 3).reshape(B, H, W, C)
```

```python
import jax
import jax.numpy as jnp
from jax import lax
import jax.experimental.pallas as pl
import jax.experimental.pallas.tpu as pltpu

_SLAB = 4096
_PIECE = 64
_R_SLABS = 18
_R_SPLIT = (2, 1)
_R_LAG = 26
_R_TAIL = 15
_R_HEAD = 72
_W_SLABS = 6
_W_FIRST = 40
_CHUNK = 768
_R_STEP = (13, 16)
_W_STEP = (7, 22)


def _upper(shape):
    return lax.broadcasted_iota(jnp.int32, shape, 1) < 4


def _tiles_to_pixels(v):
    n = v.shape[0] // 48
    u = pltpu.bitcast(v, jnp.int32).reshape(n, 24, 128)
    a, b, c = u[:, 0:8], u[:, 8:16], u[:, 16:24]
    up = _upper(a.shape)
    cols = [jnp.where(up, a, b), pltpu.roll(jnp.where(up, c, a), 4, 1), jnp.where(up, b, c)]
    return jnp.concatenate(
        [pltpu.bitcast(t.reshape(8 * n, 128), v.dtype) for t in cols], axis=1)


def _pixels_to_tiles(r):
    n = r.shape[0] // 16
    c0, c1, c2 = (
        pltpu.bitcast(r[:, i * 128:(i + 1) * 128], jnp.int32).reshape(n, 8, 128)
        for i in range(3))
    up = _upper(c0.shape)
    c1 = pltpu.roll(c1, 4, 1)
    u = jnp.concatenate(
        [jnp.where(up, c0, c1), jnp.where(up, c2, c0), jnp.where(up, c1, c2)], axis=1)
    return pltpu.bitcast(u.reshape(24 * n, 128), r.dtype)


def _share(total, parts, i):
    return range(i * total // parts, (i + 1) * total // parts)


@jax.jit
def pallas_standalone__dilated_atrous__vision_kernel(
    x: jax.Array,
    w: jax.Array,
):
    B, H, W, C = x.shape
    assert w.shape == (1, 1, C, C) and C == 3 * 128 and x.dtype.itemsize == 2
    M = B * H * W
    N = 3 * M
    n_slabs = N // _SLAB
    pieces = _SLAB // _PIECE
    turns = _R_SLABS // sum(_R_SPLIT)
    block = _R_SLABS * _SLAB
    n_blocks = N // block
    n_rounds = n_blocks * pieces
    n_writes = n_slabs // _W_SLABS * pieces
    r_chunks, r_rounds = _R_STEP
    w_chunks, w_writes = _W_STEP
    r_steps = (n_rounds - _R_HEAD - 1) // r_rounds
    r_rows = r_steps * r_chunks * _CHUNK
    w_steps = (N - r_rows) // (w_chunks * _CHUNK)
    lag_rounds, tail_rounds = pl.cdiv(_R_LAG, turns), pl.cdiv(_R_TAIL, turns)
    last_rounds = _R_HEAD + r_steps * r_rounds
    assert n_blocks * block == N and n_slabs % _W_SLABS == 0 and _CHUNK % 48 == 0
    assert turns * sum(_R_SPLIT) == _R_SLABS and last_rounds + tail_rounds <= n_rounds
    assert r_rows + w_steps * w_chunks * _CHUNK == N and r_chunks * _CHUNK <= block
    for i in range(r_steps):
        g = ((i + 1) * r_chunks * _CHUNK - 1) // block
        assert (g + 1) * pieces + lag_rounds <= _R_HEAD + i * r_rounds
    for t in range(w_steps):
        done = r_rows + t * w_chunks * _CHUNK
        assert _W_FIRST + (t + 1) * w_writes <= done // (_W_SLABS * _SLAB) * pieces

    def kernel_function(x_hbm, w_hbm, o_hbm, buf, wbuf):
        slabs = buf.reshape(n_slabs, _SLAB, 128)

        def matmuls(base, count, between):
            def rows(s):
                return pl.ds(pl.multiple_of(base + s * _CHUNK, _CHUNK), _CHUNK)

            nxt = _tiles_to_pixels(buf[rows(0)])
            for s in range(count):
                res = jnp.dot(nxt, wbuf[...], preferred_element_type=jnp.float32)
                if s + 1 < count:
                    nxt = _tiles_to_pixels(buf[rows(s + 1)])
                between(s)
                buf[rows(s)] = _pixels_to_tiles(res.astype(buf.dtype))

        def wait_rows(rows, sem):
            total = buf.at[pl.ds(0, rows)]
            pltpu.make_async_copy(total, total, sem).wait()

        def piece(k):
            g = lax.div(k, pieces)
            return g, pl.ds(pl.multiple_of((k - g * pieces) * _PIECE, _PIECE), _PIECE)

        def phases(block_sems, side_sem, out_sem):
            def start_read(r, turn, queue, sem=None):
                more, slot = divmod(turn if queue else turn - _R_LAG, turns)
                g, rows = piece(r + more)
                first = slot * sum(_R_SPLIT) + (0 if queue else _R_SPLIT[0])
                idx = (pl.ds(g * _R_SLABS + first, _R_SPLIT[1 - queue]), rows)
                sem = block_sems.at[g] if sem is None else sem
                pltpu.make_async_copy(x_hbm.at[idx], slabs.at[idx], sem).start(priority=queue)

            def start_turns(r, which):
                for turn in which:
                    start_read(r, turn, 1)
                    start_read(r, turn, 0)

            def start_write(k):
                g, rows = piece(k)
                idx = (pl.ds(g * _W_SLABS, _W_SLABS), rows)
                pltpu.make_async_copy(slabs.at[idx], o_hbm.at[idx], out_sem).start(priority=1)

            w_copy = pltpu.make_async_copy(w_hbm, wbuf, side_sem)
            w_copy.start()
            for turn in range(_R_LAG):
                start_read(jnp.int32(0), turn, 1)
            start_turns(jnp.int32(0), range(_R_LAG, lag_rounds * turns))
            pl.loop(lag_rounds, _R_HEAD)(lambda r: start_turns(r, range(turns)))
            w_copy.wait()
            wait_rows(block, block_sems.at[0])

            @pl.loop(0, r_steps)
            def _(i):
                base = i * (r_chunks * _CHUNK)
                g = lax.div(base + r_chunks * _CHUNK - 1, block)

                @pl.when(g * block >= jnp.maximum(base, 1))
                def _():
                    wait_rows(block, block_sems.at[g])

                matmuls(base, r_chunks, lambda s: start_turns(
                    _R_HEAD + i * r_rounds, _share(r_rounds * turns, r_chunks, s)))

            pl.loop(last_rounds, n_rounds - tail_rounds)(
                lambda r: start_turns(r, range(turns)))
            end = jnp.int32(n_rounds)
            for turn in range(-tail_rounds * turns, 0):
                start_read(end, turn, 1, side_sem if turn >= -_R_TAIL else None)
                start_read(end, turn, 0)
            for turn in range(_R_LAG):
                start_read(end, turn, 0)
            tail_rows = _R_TAIL * _R_SPLIT[0] * _PIECE
            for g in range((r_rows - 1) // block + 1, n_blocks - 1):
                wait_rows(block, block_sems.at[g])
            wait_rows(block - tail_rows, block_sems.at[n_blocks - 1])
            pl.loop(0, _W_FIRST)(start_write)
            wait_rows(tail_rows, side_sem)

            @pl.loop(0, w_steps)
            def _(t):
                def start_writes(s):
                    for k in _share(w_writes, w_chunks, s):
                        start_write(_W_FIRST + t * w_writes + k)

                matmuls(r_rows + t * (w_chunks * _CHUNK), w_chunks, start_writes)

            pl.loop(_W_FIRST + w_steps * w_writes, n_writes)(start_write)
            pltpu.make_async_copy(slabs, o_hbm, out_sem).wait()

        pl.run_scoped(
            phases,
            pltpu.SemaphoreType.DMA((n_blocks,)),
            pltpu.SemaphoreType.DMA(()),
            pltpu.SemaphoreType.DMA(()),
        )

    tiles = x.reshape(M // 8, 8, 3, 128).transpose(0, 2, 1, 3)
    out = pl.pallas_call(
        kernel_function,
        in_specs=[
            pl.BlockSpec(memory_space=pl.ANY),
            pl.BlockSpec(memory_space=pl.ANY),
        ],
        out_specs=pl.BlockSpec(memory_space=pl.ANY),
        out_shape=jax.ShapeDtypeStruct((n_slabs, _SLAB, 128), x.dtype),
        scratch_shapes=[
            pltpu.VMEM((N, 128), x.dtype),
            pltpu.VMEM((C, C), w.dtype),
        ],
        compiler_params=pltpu.CompilerParams(
            vmem_limit_bytes=120 * 2**20, disable_bounds_checks=True),
    )(tiles.reshape(n_slabs, _SLAB, 128), w.reshape(C, C))
    return out.reshape(M // 8, 3, 8, 128).transpose(0, 2, 1, 3).reshape(B, H, W, C)
```

```python
import jax
import jax.numpy as jnp
from jax import lax
import jax.experimental.pallas as pl
import jax.experimental.pallas.tpu as pltpu

_SLAB = 4096
_PIECE = 64
_R_SLABS = 18
_R_SPLIT = (2, 1)
_R_LAG = 26
_R_TAIL = 15
_R_HEAD = 72
_W_SLABS = 6
_W_FIRST = 54
_CHUNK = 768
_R_STEP = (13, 16)
_W_STEP = (7, 22)


def _upper(shape):
    return lax.broadcasted_iota(jnp.int32, shape, 1) < 4


def _tiles_to_pixels(v):
    n = v.shape[0] // 48
    u = pltpu.bitcast(v, jnp.int32).reshape(n, 24, 128)
    a, b, c = u[:, 0:8], u[:, 8:16], u[:, 16:24]
    up = _upper(a.shape)
    cols = [jnp.where(up, a, b), pltpu.roll(jnp.where(up, c, a), 4, 1), jnp.where(up, b, c)]
    return jnp.concatenate(
        [pltpu.bitcast(t.reshape(8 * n, 128), v.dtype) for t in cols], axis=1)


def _pixels_to_tiles(r):
    n = r.shape[0] // 16
    c0, c1, c2 = (
        pltpu.bitcast(r[:, i * 128:(i + 1) * 128], jnp.int32).reshape(n, 8, 128)
        for i in range(3))
    up = _upper(c0.shape)
    c1 = pltpu.roll(c1, 4, 1)
    u = jnp.concatenate(
        [jnp.where(up, c0, c1), jnp.where(up, c2, c0), jnp.where(up, c1, c2)], axis=1)
    return pltpu.bitcast(u.reshape(24 * n, 128), r.dtype)


def _share(total, parts, i):
    return range(i * total // parts, (i + 1) * total // parts)


@jax.jit
def pallas_standalone__dilated_atrous__vision_kernel(
    x: jax.Array,
    w: jax.Array,
):
    B, H, W, C = x.shape
    assert w.shape == (1, 1, C, C) and C == 3 * 128 and x.dtype.itemsize == 2
    M = B * H * W
    N = 3 * M
    n_slabs = N // _SLAB
    pieces = _SLAB // _PIECE
    turns = _R_SLABS // sum(_R_SPLIT)
    block = _R_SLABS * _SLAB
    n_blocks = N // block
    n_rounds = n_blocks * pieces
    n_writes = n_slabs // _W_SLABS * pieces
    r_chunks, r_rounds = _R_STEP
    w_chunks, w_writes = _W_STEP
    r_steps = (n_rounds - _R_HEAD - 1) // r_rounds
    r_rows = r_steps * r_chunks * _CHUNK
    w_steps = (N - r_rows) // (w_chunks * _CHUNK)
    lag_rounds, tail_rounds = pl.cdiv(_R_LAG, turns), pl.cdiv(_R_TAIL, turns)
    last_rounds = _R_HEAD + r_steps * r_rounds
    assert n_blocks * block == N and n_slabs % _W_SLABS == 0 and _CHUNK % 48 == 0
    assert turns * sum(_R_SPLIT) == _R_SLABS and last_rounds + tail_rounds <= n_rounds
    assert r_rows + w_steps * w_chunks * _CHUNK == N and r_chunks * _CHUNK <= block
    for i in range(r_steps):
        g = ((i + 1) * r_chunks * _CHUNK - 1) // block
        assert (g + 1) * pieces + lag_rounds <= _R_HEAD + i * r_rounds
    for t in range(w_steps):
        done = r_rows + t * w_chunks * _CHUNK
        assert _W_FIRST + (t + 1) * w_writes <= done // (_W_SLABS * _SLAB) * pieces

    def kernel_function(x_hbm, w_hbm, o_hbm, buf, wbuf):
        slabs = buf.reshape(n_slabs, _SLAB, 128)

        def matmuls(base, count, between):
            def rows(s):
                return pl.ds(pl.multiple_of(base + s * _CHUNK, _CHUNK), _CHUNK)

            weights = wbuf[...]
            nxt = _tiles_to_pixels(buf[rows(0)])
            for s in range(count):
                res = jnp.dot(nxt, weights, preferred_element_type=jnp.float32)
                if s + 1 < count:
                    nxt = _tiles_to_pixels(buf[rows(s + 1)])
                between(s)
                buf[rows(s)] = _pixels_to_tiles(res.astype(buf.dtype))

        def wait_all(size_of, sem):
            pltpu.make_async_copy(size_of, size_of, sem).wait()

        def piece(k):
            g = lax.div(k, pieces)
            return g, pl.ds(pl.multiple_of((k - g * pieces) * _PIECE, _PIECE), _PIECE)

        def phases(block_sems, side_sem, out_sem):
            def start_read(r, turn, queue, sem=None):
                more, slot = divmod(turn if queue else turn - _R_LAG, turns)
                g, rows = piece(r + more)
                first = slot * sum(_R_SPLIT) + (0 if queue else _R_SPLIT[0])
                idx = (pl.ds(g * _R_SLABS + first, _R_SPLIT[1 - queue]), rows)
                sem = block_sems.at[g] if sem is None else sem
                pltpu.make_async_copy(x_hbm.at[idx], slabs.at[idx], sem).start(priority=queue)

            def start_turns(r, which):
                for turn in which:
                    start_read(r, turn, 1)
                    start_read(r, turn, 0)

            def wait_block(g):
                wait_all(slabs.at[pl.ds(g * _R_SLABS, _R_SLABS)], block_sems.at[g])

            def start_write(k):
                g, rows = piece(k)
                idx = (pl.ds(g * _W_SLABS, _W_SLABS), rows)
                pltpu.make_async_copy(slabs.at[idx], o_hbm.at[idx], out_sem).start(priority=1)

            w_copy = pltpu.make_async_copy(w_hbm, wbuf, side_sem)
            w_copy.start()
            for turn in range(_R_LAG):
                start_read(0, turn, 1)
            start_turns(0, range(_R_LAG, lag_rounds * turns))
            pl.loop(lag_rounds, _R_HEAD)(lambda r: start_turns(r, range(turns)))
            w_copy.wait()
            wait_block(0)

            @pl.loop(0, r_steps)
            def _(i):
                base = i * (r_chunks * _CHUNK)
                g = lax.div(base + r_chunks * _CHUNK - 1, block)

                @pl.when(g * block >= jnp.maximum(base, 1))
                def _():
                    wait_block(g)

                matmuls(base, r_chunks, lambda s: start_turns(
                    _R_HEAD + i * r_rounds, _share(r_rounds * turns, r_chunks, s)))

            pl.loop(last_rounds, n_rounds - tail_rounds)(
                lambda r: start_turns(r, range(turns)))
            for turn in range(-tail_rounds * turns, 0):
                start_read(n_rounds, turn, 1, side_sem if turn >= -_R_TAIL else None)
                start_read(n_rounds, turn, 0)
            for turn in range(_R_LAG):
                start_read(n_rounds, turn, 0)
            tail_rows = _R_TAIL * _R_SPLIT[0] * _PIECE
            for g in range((r_rows - 1) // block + 1, n_blocks - 1):
                wait_block(g)
            wait_all(buf.at[pl.ds(0, block - tail_rows)], block_sems.at[n_blocks - 1])
            pl.loop(0, _W_FIRST)(start_write)
            wait_all(buf.at[pl.ds(0, tail_rows)], side_sem)

            @pl.loop(0, w_steps)
            def _(t):
                def start_writes(s):
                    for k in _share(w_writes, w_chunks, s):
                        start_write(_W_FIRST + t * w_writes + k)

                matmuls(r_rows + t * (w_chunks * _CHUNK), w_chunks, start_writes)

            pl.loop(_W_FIRST + w_steps * w_writes, n_writes)(start_write)
            pltpu.make_async_copy(slabs, o_hbm, out_sem).wait()

        pl.run_scoped(
            phases,
            pltpu.SemaphoreType.DMA((n_blocks,)),
            pltpu.SemaphoreType.DMA(()),
            pltpu.SemaphoreType.DMA(()),
        )

    tiles = x.reshape(M // 8, 8, 3, 128).transpose(0, 2, 1, 3)
    out = pl.pallas_call(
        kernel_function,
        in_specs=[
            pl.BlockSpec(memory_space=pl.ANY),
            pl.BlockSpec(memory_space=pl.ANY),
        ],
        out_specs=pl.BlockSpec(memory_space=pl.ANY),
        out_shape=jax.ShapeDtypeStruct((n_slabs, _SLAB, 128), x.dtype),
        scratch_shapes=[
            pltpu.VMEM((N, 128), x.dtype),
            pltpu.VMEM((C, C), w.dtype),
        ],
        compiler_params=pltpu.CompilerParams(
            vmem_limit_bytes=120 * 2**20, disable_bounds_checks=True),
    )(tiles.reshape(n_slabs, _SLAB, 128), w.reshape(C, C))
    return out.reshape(M // 8, 3, 8, 128).transpose(0, 2, 1, 3).reshape(B, H, W, C)
```
